```python
import jax
import jax.numpy as jnp

def _softmax(x, axis=-1):
    return jax.nn.softmax(x, axis=axis)
def _gelu(x):
    return jax.nn.gelu(x, approximate=True)
def _silu(x):
    return jax.nn.silu(x)
def _sigmoid(x):
    return jax.nn.sigmoid(x)
def _layernorm(x, axis=-1, eps=1e-5):
    m = jnp.mean(x, axis=axis, keepdims=True)
    v = jnp.var(x, axis=axis, keepdims=True)
    return (x - m) / jnp.sqrt(v + eps)
def _scatter_add(tgt, idx, src, axis=0):
    return tgt.at[idx].add(src)
def _segment_sum(src, seg, n):
    return jax.ops.segment_sum(src, seg, n)
class _Rng:
    def __init__(self, key):
        self._k = key
    def _next(self):
        self._k, sub = jax.random.split(self._k)
        return sub
    def normal(self, shape):
        return jax.random.normal(self._next(), shape, dtype=jnp.bfloat16)
    def randint(self, lo, hi, shape):
        return jax.random.randint(self._next(), shape, lo, hi, dtype=jnp.int32)
    def uniform(self, shape, lo=0.0, hi=1.0):
        return jax.random.uniform(self._next(), shape, jnp.bfloat16, lo, hi)
    def permutation(self, n):
        return jax.random.permutation(self._next(), n)


kernel_name = 'sequential_preLN__grouped_kv_mqa__glu_gated_swiglu__prompt'

def _fwd_setup_inputs():
    _rng = _Rng(jax.random.key(int.from_bytes(__import__("os").urandom(4), "little")))
    _w = (lambda a: (lambda t: t.astype(jnp.bfloat16) if jnp.issubdtype(t.dtype, jnp.floating) else t)(jnp.asarray(a)))
    def _A_setup():
        B, S, D, H = 1, 2048, 512, 32
        Dh = D // H
        return {
            "x": _w((lambda *s: _rng.normal(s) * 0.05)(B, S, D)),
            "wq": _w((lambda *s: _rng.normal(s) * 0.05)(D, H * Dh)),
            "wk": _w((lambda *s: _rng.normal(s) * 0.05)(D, Dh)),
            "wv": _w((lambda *s: _rng.normal(s) * 0.05)(D, Dh)),
            "wo": _w((lambda *s: _rng.normal(s) * 0.05)(H * Dh, D)),
        }
    _A_in = _A_setup()

    def _B_setup():
        B, S, D, F = 1, 2048, 512, 1376
        return {
            "x": _w((lambda *s: _rng.normal(s) * 0.05)(B, S, D)),
            "w1": _w((lambda *s: _rng.normal(s) * 0.05)(D, F) * (2.0 / D) ** 0.5),
            "w3": _w((lambda *s: _rng.normal(s) * 0.05)(D, F) * (2.0 / D) ** 0.5),
            "w2": _w((lambda *s: _rng.normal(s) * 0.05)(F, D) * (2.0 / F) ** 0.5),
        }
    _B_in = _B_setup()

    return {
        "A_x": _A_in["x"],
        "A_wq": _A_in["wq"],
        "A_wk": _A_in["wk"],
        "A_wv": _A_in["wv"],
        "A_wo": _A_in["wo"],
        "B_x": _B_in["x"],
        "B_w1": _B_in["w1"],
        "B_w3": _B_in["w3"],
        "B_w2": _B_in["w2"],
    }

def _fwd_reference(A_x, A_wq, A_wk, A_wv, A_wo, B_x, B_w1, B_w3, B_w2):
    def _A_ref(x, wq, wk, wv, wo):
        B, S, D = x.shape
        H = 32
        Dh = D // H
        q = (lambda x, *d: x.transpose(*d))((x @ wq).reshape(B, S, H, Dh), 0, 2, 1, 3)
        k = x @ wk
        v = x @ wv
        scores = jnp.einsum("bhqd,bkd->bhqk", q, k) * (Dh ** -0.5)
        p = _softmax(scores, axis=-1)
        o = jnp.einsum("bhqk,bkd->bhqd", p, v)
        return (lambda x, *d: x.transpose(*d))(o, 0, 2, 1, 3).reshape(B, S, H * Dh) @ wo

    def _B_ref(x, w1, w3, w2):
        gate = jnp.einsum("bsd,df->bsf", x, w1)
        up = jnp.einsum("bsd,df->bsf", x, w3)
        h = _silu(gate) * up
        out = jnp.einsum("bsf,fd->bsd", h, w2)
        return out

    x = A_x
    h = x + _A_ref(_layernorm(x, axis=-1), A_wq, A_wk, A_wv, A_wo)
    h2 = h + _B_ref(_layernorm(h, axis=-1), B_w1, B_w3, B_w2)
    return h2


def setup_inputs():
    _inp = _fwd_setup_inputs()
    _gk = jax.random.fold_in(jax.random.key(int.from_bytes(__import__("os").urandom(4), "little")), 2**31 - 1)
    _shapes = [[1, 2048, 512]]
    _dtypes = ['bfloat16']
    _gks = jax.random.split(_gk, len(_shapes))
    _gs = [jax.random.normal(k, s, dtype=jnp.dtype(d)) * 0.05 for k, s, d in zip(_gks, _shapes, _dtypes)]
    _inp["grad_out"] = _gs[0]
    return _inp

def reference(A_x, A_wq, A_wk, A_wv, A_wo, B_w1, B_w3, B_w2, B_x, grad_out):
    _const = dict(B_x=B_x)
    def _f(*_d):
        return _fwd_reference(**{'A_x': _d[0], 'A_wq': _d[1], 'A_wk': _d[2], 'A_wv': _d[3], 'A_wo': _d[4], 'B_w1': _d[5], 'B_w3': _d[6], 'B_w2': _d[7], **_const})
    _out, _vjp = jax.vjp(_f, A_x, A_wq, A_wk, A_wv, A_wo, B_w1, B_w3, B_w2)
    _grads = _vjp(grad_out)
    _out0 = jnp.asarray(_out)
    return (_out0, *[jnp.asarray(_g) for _g in _grads])
```

```python
import jax
import jax.numpy as jnp
from jax import lax
import jax.experimental.pallas as pl
import jax.experimental.pallas.tpu as pltpu

S, D, H, DH, F = 2048, 512, 32, 16, 1376
BQ = 128
NQ = S // BQ
GH = 4
NG = H // GH
GW = GH * BQ
NC = S // 128
EPS = 1e-5
LOG2E = 1.4426950408889634
QSCALE = (DH ** -0.5) * LOG2E

bf = jnp.bfloat16
f32 = jnp.float32
u32 = jnp.uint32
NT = (((1,), (1,)), ((), ()))


def _dot(a, b):
    return jnp.dot(a, b, preferred_element_type=f32)


def _dnt(a, b):
    return lax.dot_general(a, b, NT, preferred_element_type=f32)


def _split2(x):
    r, w = x.shape
    x4 = x.reshape(r // 16, 2, 8, w)
    return x4[:, 0].reshape(r // 2, w), x4[:, 1].reshape(r // 2, w)


def _pack2(a, b):
    return pltpu.pack_elementwise([a, b], packed_dtype=bf)


def _unpack2(x):
    return (pltpu.unpack_elementwise(x, index=0, packed_dtype=bf, unpacked_dtype=f32),
            pltpu.unpack_elementwise(x, index=1, packed_dtype=bf, unpacked_dtype=f32))


def _ln_t(xt):
    mean = jnp.mean(xt, axis=0, keepdims=True)
    xc = xt - mean
    var = jnp.mean(xc * xc, axis=0, keepdims=True)
    rstd = lax.rsqrt(var + EPS)
    return xc * rstd, rstd


def _ln_bwd_t(dy, xhat, rstd):
    m1 = jnp.mean(dy, axis=0, keepdims=True)
    m2 = jnp.mean(dy * xhat, axis=0, keepdims=True)
    return rstd * (dy - m1 - xhat * m2)


def _kernel(x_ref, wq_ref, wkT_ref, wvT_ref, wo_ref, w1T, w3T, w2_ref, g_ref,
            h2_ref, dx_ref, dwq_ref, dwkT_ref, dwvT_ref, dwo_ref, dw1T_ref, dw3T_ref, dw2_ref,
            wqT, woT, w1_s, w3_s, w2T, wkv_s,
            xn_s, kp_s, vp_s, kt_s, vt_s,
            sA, sB, p_s, ds_s,
            qt_s, do_s, dl_s, o_s, li_s, dq_s,
            dkt_s, dvt_s, dh_s, dxq_s,
            ot_s, hh_s, dg_s, du_s, dhh_s, dqt_s,
            dwq_a, dwo_a, dw1_a, dw3_a, dw2_a):
    i = pl.program_id(0)

    @pl.when(i == 0)
    def _prologue():
        wqT[...] = wq_ref[...].T
        woT[...] = wo_ref[...].T
        w1_s[...] = w1T[...].T
        w3_s[...] = w3T[...].T
        w2T[...] = w2_ref[...].T
        wkvT = jnp.concatenate([wkT_ref[...], wvT_ref[...]], axis=0)
        wkv_s[...] = wkvT.astype(f32).T.astype(bf)
        r = lax.broadcasted_iota(jnp.int32, (128, 128), 0)
        c = lax.broadcasted_iota(jnp.int32, (128, 128), 1)
        rr = r % 16
        key = (r - rr) + jnp.where(rr < 8, 2 * rr, 2 * (rr - 8) + 1)
        perm = jnp.where(c == key, 1.0, 0.0).astype(bf)

        def blk(jj, carry):
            for t in range(4):
                j = jj * 4 + t
                xt = x_ref[pl.ds(pl.multiple_of(j * BQ, BQ), BQ), :].astype(f32).T
                xh, _ = _ln_t(xt)
                xn_s[j] = xh.astype(bf)
            return carry
        lax.fori_loop(0, NQ // 4, blk, 0)
        for j in range(NQ):
            kv = _dot(wkvT, xn_s[j]).astype(bf)
            kt_s[j] = kv[0:16]
            vt_s[j] = kv[16:32]
        for j in range(NQ):
            kp_s[j] = _dnt(perm, kt_s[j]).astype(bf)
            vp_s[j] = _dnt(perm, vt_s[j]).astype(bf)
        qT = (_dot(wqT[...], xn_s[0]) * QSCALE).astype(bf)
        for g in range(NG):
            qt_s[g] = jnp.concatenate([qT[64 * g + 16 * j:64 * g + 16 * j + 16] for j in range(GH)], axis=1)
        dkt_s[...] = jnp.zeros(dkt_s.shape, f32)
        dvt_s[...] = jnp.zeros(dvt_s.shape, f32)
        dwq_a[...] = jnp.zeros(dwq_a.shape, f32)
        dwo_a[...] = jnp.zeros(dwo_a.shape, f32)
        dw1_a[...] = jnp.zeros(dw1_a.shape, f32)
        dw3_a[...] = jnp.zeros(dw3_a.shape, f32)
        dw2_a[...] = jnp.zeros(dw2_a.shape, f32)
        ds_s[...] = jnp.zeros(ds_s.shape, u32)
        dqt_s[...] = jnp.zeros(dqt_s.shape, bf)
        dq_s[...] = jnp.zeros(dq_s.shape, f32)

    def pass1_chunk(qt, sref, c, m):
        rows = slice(c * 128, (c + 1) * 128)
        s = _dot(kp_s[c], qt)
        sref[rows, :] = s
        return jnp.maximum(m, jnp.max(s.reshape(16, 8, GW), axis=0))

    def pass2_chunk(g, sref, c, m, o, l):
        rows = slice(c * 128, (c + 1) * 128)
        rows2 = slice(c * 64, (c + 1) * 64)
        p = jnp.exp2(sref[rows, :] - m)
        l = l + jnp.sum(p.reshape(16, 8, GW), axis=0)
        pi = _pack2(*_split2(p))
        p_s[g, rows2, :] = pi
        o = o + _dot(vt_s[c], pltpu.bitcast(pi, bf))
        return o, l

    row0 = pl.multiple_of(i * BQ, BQ)
    gt32 = g_ref[pl.ds(row0, BQ), :].astype(f32).T
    gt = gt32.astype(bf)

    def dhh_chunk(n):
        r0 = n * 128
        r1 = min(r0 + 128, F)
        dhh_s[r0:r1, :] = _dot(w2_ref[r0:r1, :], gt)

    def step(g, m, sread, swrite, do1=True, do2=True, filler=None):
        if do2:
            mrow = jnp.max(m, axis=0, keepdims=True)
        if do1:
            qt = qt_s[g + 1]
        m2 = jnp.full((8, GW), -jnp.inf, f32)
        l = jnp.zeros((8, GW), f32)
        o = jnp.zeros((16, GW), f32)
        for c in range(NC):
            if do1:
                m2 = pass1_chunk(qt, swrite, c, m2)
            if do2:
                o, l = pass2_chunk(g, sread, c, mrow, o, l)
            if filler is not None:
                filler(c)
        if do2:
            linv = 1.0 / jnp.sum(l, axis=0, keepdims=True)
            o_s[g] = o * linv
            li_s[g] = jnp.broadcast_to(linv, (8, GW))
        return m2

    m = step(-1, None, None, sA, do2=False)

    def fbody(gg, m):
        m = step(2 * gg, m, sA, sB)
        m = step(2 * gg + 1, m, sB, sA)
        return m
    m = lax.fori_loop(0, NG // 2 - 1, fbody, m)
    m = step(NG - 2, m, sA, sB)
    step(NG - 1, m, sB, None, do1=False, filler=lambda c: dhh_chunk(c - 5) if c >= 5 else None)

    def to_rows(src, scale):
        for g in range(NG):
            og = (src[g] * scale).astype(bf) if scale != 1.0 else src[g].astype(bf)
            for j in range(GH):
                yield 64 * g + 16 * j, og[:, 128 * j:128 * (j + 1)]

    for r0, v in to_rows(o_s, 1.0):
        ot_s[r0:r0 + 16, :] = v
    ot = ot_s[...]
    xt = x_ref[pl.ds(row0, BQ), :].astype(f32).T
    h = xt + _dot(woT[...], ot)

    def dx_q_part(j):
        dqt = dqt_s[...]
        dxq_s[jnp.maximum(j, 0)] = _dot(wq_ref[...], dqt)
        dwq_a[...] += _dnt(xn_s[jnp.maximum(j, 0)], dqt)
    dx_q_part(i - 1)

    hhat, rstd2 = _ln_t(h)
    hn = hhat.astype(bf)

    for r0 in range(0, F, 128):
        r1 = min(r0 + 128, F)
        gate = _dot(w1T[r0:r1, :], hn)
        up = _dot(w3T[r0:r1, :], hn)
        dhh = dhh_s[r0:r1, :]
        sig = jax.nn.sigmoid(gate)
        silu = gate * sig
        hh_s[r0:r1, :] = (silu * up).astype(bf)
        du_s[r0:r1, :] = (dhh * silu).astype(bf)
        dg_s[r0:r1, :] = (dhh * up * (sig + silu * (1.0 - sig))).astype(bf)

    hh = hh_s[...]
    dg = dg_s[...]
    du = du_s[...]
    dhn = _dot(w1_s[...], dg) + _dot(w3_s[...], du)
    h2 = h + _dot(w2T[...], hh)
    h2_ref[...] = h2.T.astype(bf)
    dw2_a[...] += _dnt(hh, gt)
    dh = gt32 + _ln_bwd_t(dhn, hhat, rstd2)
    dh_s[i] = dh
    dhb = dh.astype(bf)
    dO = _dot(wo_ref[...], dhb)
    dwo_a[...] += _dnt(ot, dhb)
    dw1_a[...] += _dnt(dg, hn)
    for g in range(NG):
        dog = jnp.concatenate([dO[64 * g + 16 * j:64 * g + 16 * j + 16] for j in range(GH)], axis=1)
        dob = (dog * li_s[g, 0:1, :]).astype(bf)
        do_s[g] = dob
        dl_s[g] = jnp.broadcast_to(jnp.sum(dob.astype(f32) * o_s[g], axis=0, keepdims=True), (8, GW))

    def A(g, dOg, delta, c, half):
        r2 = slice(c * 64 + half * 32, c * 64 + half * 32 + 32)
        dp = _dot(vp_s[c, half * 64:half * 64 + 64, :], dOg)
        pa, pb = _unpack2(p_s[g, r2, :])
        da, db = _split2(dp)
        ds_s[c % 4, half * 32:half * 32 + 32, :] = _pack2(pa * (da - delta), pb * (db - delta))

    def Bq(c, dq):
        return dq + _dot(kt_s[c], pltpu.bitcast(ds_s[c % 4], bf))

    def Bk(qt, c):
        dkt_s[c] += _dnt(qt, pltpu.bitcast(ds_s[c % 4], bf))

    def Bv(g, dOg, c):
        dvt_s[c] += _dnt(dOg, pltpu.bitcast(p_s[g, c * 64:(c + 1) * 64, :], bf))

    LAG = 2

    def bbody(g, dq_prev):
        gp = jnp.maximum(g - 1, 0)
        valid = g > 0
        qt = qt_s[g]
        dOg = do_s[g]
        delta = dl_s[g, 0:1, :]
        qt_p = jnp.where(valid, qt_s[gp], jnp.zeros((DH, GW), bf))
        dO_p = jnp.where(valid, do_s[gp], jnp.zeros((DH, GW), bf))
        dq = jnp.zeros((DH, GW), f32)
        for it in range(NC):
            c = it - LAG
            A(g, dOg, delta, it, 0)
            if c < 0:
                Bv(gp, dO_p, NC + c)
            else:
                Bv(g, dOg, c)
            A(g, dOg, delta, it, 1)
            if c < 0:
                Bk(qt_p, NC + c)
                dq_prev = Bq(NC + c, dq_prev)
                if c == -1:
                    dq_s[gp] = dq_prev
            else:
                Bk(qt, c)
                dq = Bq(c, dq)
        return dq
    dq = lax.fori_loop(0, NG, bbody, jnp.zeros((DH, GW), f32))
    qt_l = qt_s[NG - 1]
    dO_l = do_s[NG - 1]
    qn = (_dot(wqT[...], xn_s[jnp.minimum(i + 1, NQ - 1)]) * QSCALE).astype(bf)
    for c in range(NC - LAG, NC):
        Bv(NG - 1, dO_l, c)
        Bk(qt_l, c)
        dq = Bq(c, dq)
    dq_s[NG - 1] = dq
    dw3_a[...] += _dnt(du, hn)
    for g in range(NG):
        qt_s[g] = jnp.concatenate([qn[64 * g + 16 * j:64 * g + 16 * j + 16] for j in range(GH)], axis=1)
    for r0, v in to_rows(dq_s, DH ** -0.5):
        dqt_s[r0:r0 + 16, :] = v

    @pl.when(i == NQ - 1)
    def _epilogue():
        dx_q_part(NQ - 1)
        wkv = wkv_s[...]

        def blk(jj, acc):
            dkvs = []
            for t in range(2):
                j = jj * 2 + t
                dkvs.append(jnp.concatenate([(dkt_s[j] * (1.0 / LOG2E)).astype(bf), dvt_s[j].astype(bf)], axis=0))
            dxns = [dxq_s[jj * 2 + t] + _dot(wkv, dkvs[t]) for t in range(2)]
            for t in range(2):
                acc = acc + _dnt(dkvs[t], xn_s[jj * 2 + t])
            for t in range(2):
                j = jj * 2 + t
                r = pl.ds(pl.multiple_of(j * BQ, BQ), BQ)
                xt = x_ref[r, :].astype(f32).T
                xh, rstd = _ln_t(xt)
                dx = dh_s[j] + _ln_bwd_t(dxns[t], xh, rstd)
                dx_ref[r, :] = dx.T.astype(bf)
            return acc
        acc = lax.fori_loop(0, NQ // 2, blk, jnp.zeros((32, D), f32))
        dwkT_ref[...] = acc[0:16].astype(bf)
        dwvT_ref[...] = acc[16:32].astype(bf)
        dwq_ref[...] = dwq_a[...].astype(bf)
        dwo_ref[...] = dwo_a[...].astype(bf)
        dw1T_ref[...] = dw1_a[...].astype(bf)
        dw3T_ref[...] = dw3_a[...].astype(bf)
        dw2_ref[...] = dw2_a[...].astype(bf)


def _full(shape):
    return pl.BlockSpec(shape, lambda i, n=len(shape): (0,) * n)


@jax.jit
def pallas_sequential_preLN__grouped_kv_mqa__glu_gated_swiglu__prompt_kernel(
    A_x: jax.Array,
    A_wq: jax.Array,
    A_wk: jax.Array,
    A_wv: jax.Array,
    A_wo: jax.Array,
    B_x: jax.Array,
    B_w1: jax.Array,
    B_w3: jax.Array,
    B_w2: jax.Array,
    grad_out: jax.Array,
):
    del B_x
    x = A_x.reshape(S, D)
    g = grad_out.reshape(S, D)
    ins = (x, A_wq, A_wk.T, A_wv.T, A_wo, B_w1.T, B_w3.T, B_w2, g)
    out_shapes = [(S, D), (S, D), (D, D), (DH, D), (DH, D), (D, D), (F, D), (F, D), (F, D)]
    out_specs = [pl.BlockSpec((BQ, D), lambda i: (i, 0))] + [_full(s) for s in out_shapes[1:]]
    V = pltpu.VMEM
    scratch = [
        V((D, D), bf), V((D, D), bf), V((D, F), bf), V((D, F), bf), V((D, F), bf), V((D, 32), bf),
        V((NQ, D, BQ), bf), V((NQ, 128, DH), bf), V((NQ, 128, DH), bf), V((NQ, DH, 128), bf), V((NQ, DH, 128), bf),
        V((S, GW), f32), V((S, GW), f32), V((NG, S // 2, GW), u32), V((4, 64, GW), u32),
        V((NG, DH, GW), bf), V((NG, DH, GW), bf), V((NG, 8, GW), f32), V((NG, DH, GW), f32), V((NG, 8, GW), f32),
        V((NG, DH, GW), f32),
        V((NC, DH, 128), f32), V((NC, DH, 128), f32), V((NQ, D, BQ), f32), V((NQ, D, BQ), f32),
        V((D, BQ), bf), V((F, BQ), bf), V((F, BQ), bf), V((F, BQ), bf), V((F, BQ), f32), V((D, BQ), bf),
        V((D, D), f32), V((D, D), f32), V((F, D), f32), V((F, D), f32), V((F, D), f32),
    ]
    outs = pl.pallas_call(
        _kernel,
        grid=(NQ,),
        in_specs=[_full(a.shape) for a in ins],
        out_specs=out_specs,
        out_shape=[jax.ShapeDtypeStruct(s, bf) for s in out_shapes],
        scratch_shapes=scratch,
        compiler_params=pltpu.CompilerParams(
            dimension_semantics=("arbitrary",), vmem_limit_bytes=120 * 1024 * 1024),
    )(*ins)
    h2, dx = outs[0].reshape(1, S, D), outs[1].reshape(1, S, D)
    return (h2, dx, outs[2], outs[3].T, outs[4].T, outs[5], outs[6].T, outs[7].T, outs[8])
```

```python
import jax
import jax.numpy as jnp
from jax import lax
import jax.experimental.pallas as pl
import jax.experimental.pallas.tpu as pltpu

S, D, H, DH, F = 2048, 512, 32, 16, 1376
BQ = 128
NQ = S // BQ
GW = 512
GH = GW // BQ
RG = GH * DH
NG = H // GH
NC = S // 128
EPS = 1e-5
LOG2E = 1.4426950408889634
QSCALE = (DH ** -0.5) * LOG2E
FLAG = 2
BLAG = 2
XCH = 4

bf = jnp.bfloat16
f32 = jnp.float32
u32 = jnp.uint32
NT = (((1,), (1,)), ((), ()))


def _dot(a, b):
    return jnp.dot(a, b, preferred_element_type=f32)


def _dnt(a, b):
    return lax.dot_general(a, b, NT, preferred_element_type=f32)


def _split2(x):
    r, w = x.shape
    x4 = x.reshape(r // 16, 2, 8, w)
    return x4[:, 0].reshape(r // 2, w), x4[:, 1].reshape(r // 2, w)


def _tree(op, x):
    while x.shape[0] > 8:
        h = x.shape[0] // 2
        x = op(x[:h], x[h:])
    return x


def _colmean(x):
    return jnp.sum(_tree(jnp.add, x), axis=0, keepdims=True) * (1.0 / x.shape[0])


def _pack2(a, b):
    return pltpu.pack_elementwise([a, b], packed_dtype=bf)


def _unpack2(x):
    return (pltpu.unpack_elementwise(x, index=0, packed_dtype=bf, unpacked_dtype=f32),
            pltpu.unpack_elementwise(x, index=1, packed_dtype=bf, unpacked_dtype=f32))


def _groups(x):
    return [jnp.concatenate([x[RG * g + DH * j:RG * g + DH * j + DH] for j in range(GH)], axis=1)
            for g in range(NG)]


def _ungroup(dst, src, scale):
    for g in range(NG):
        v = (src[g] * scale).astype(bf) if scale != 1.0 else src[g].astype(bf)
        for j in range(GH):
            r0 = RG * g + DH * j
            dst[r0:r0 + DH, :] = v[:, BQ * j:BQ * (j + 1)]


def _kernel(x_hbm, wq_hbm, wkT_hbm, wvT_hbm, wo_hbm, w1T_hbm, w3T_hbm, w2_hbm, g_hbm,
            h2_hbm, dx_hbm, dwq_hbm, dwkT_hbm, dwvT_hbm, dwo_hbm, dw1T_hbm, dw3T_hbm, dw2_hbm,
            x_ref, wq_ref, wkT_ref, wvT_ref, wo_ref, w1T, w3T, w2_ref, g_ref,
            h2_ref, dx_ref, dwq_ref, dwkT_ref, dwvT_ref, dwo_ref, dw1T_ref, dw3T_ref, dw2_ref,
            isem, hsem, xsem, wsem, x0sem,
            wqT, woT, w1_s, w3_s, w2T, wkv_s,
            xn_s, kp_s, vp_s, kt_s, vt_s,
            sA, sB, p_s, ds_s, qt_s, do_s, dl_s, o_s, li_s, dq_s, dkt_s, dvt_s,
            dh_s, dxq_s, xh_s, rs_s,
            ot_s, hh_s, dg_s, du_s, dhh_s, dqt_s, gt32_s, gt_s, hhat_s, hn_s, hnp_s, dhb_s, h_s, dhn_s,
            dwq_a, dwo_a, dw1_a, dw3_a, dw2_a):

    xr = S // XCH
    x_copies = [pltpu.make_async_copy(x_hbm.at[pl.ds(n * xr, xr), :], x_ref.at[pl.ds(n * xr, xr), :], x0sem.at[n])
                for n in range(XCH)]
    in_copies = [pltpu.make_async_copy(s, d, isem.at[n]) for n, (s, d) in enumerate(
        [(wkT_hbm, wkT_ref), (wvT_hbm, wvT_ref), (wq_hbm, wq_ref), (g_hbm, g_ref),
         (wo_hbm, wo_ref), (w2_hbm, w2_ref), (w1T_hbm, w1T), (w3T_hbm, w3T)])]
    w_copies = [pltpu.make_async_copy(s, d, wsem.at[n]) for n, (s, d) in enumerate(
        [(dwo_ref, dwo_hbm), (dw1T_ref, dw1T_hbm), (dw2_ref, dw2_hbm), (dw3T_ref, dw3T_hbm),
         (dwq_ref, dwq_hbm), (dwkT_ref, dwkT_hbm), (dwvT_ref, dwvT_hbm)])]

    def rows(j):
        return pl.ds(j * BQ if isinstance(j, int) else pl.multiple_of(j * BQ, BQ), BQ)

    def h2_copy(j):
        return pltpu.make_async_copy(h2_ref.at[j], h2_hbm.at[rows(j), :], hsem.at[j])

    def dx_copy(j):
        return pltpu.make_async_copy(dx_ref.at[j], dx_hbm.at[rows(j), :], xsem.at[j])

    def accum(ref, val, start):
        ref[...] = (ref[...] if start is False else jnp.where(start, 0.0, ref[...])) + val

    def load_g(j):
        gt32 = g_ref[rows(j), :].astype(f32).T
        gt32_s[...] = gt32
        gt_s[...] = gt32.astype(bf)

    def q_proj(j):
        q = (_dot(wqT[...], xn_s[j]) * QSCALE).astype(bf)
        for g, v in enumerate(_groups(q)):
            qt_s[g] = v

    def dx_q_part(j, start):
        dxq_s[j] = _dot(wq_ref[...], dqt_s[...])
        accum(dwq_a, _dnt(xn_s[j], dqt_s[...]), start)

    def pass1_chunk(qt, sref, c, m):
        s = _dot(kp_s[c], qt)
        sref[c * 128:(c + 1) * 128, :] = s
        return jnp.maximum(m, _tree(jnp.maximum, s))

    def pass2_chunk(g, sref, c, m, o, l):
        p = jnp.exp2(sref[c * 128:(c + 1) * 128, :] - m)
        pa, pb = _split2(p)
        l = l + _tree(jnp.add, pa + pb)
        pi = _pack2(pa, pb)
        p_s[g, c * 64:(c + 1) * 64, :] = pi
        o = o + _dot(vt_s[c], pltpu.bitcast(pi, bf))
        return o, l

    OFF = NC + FLAG
    NCH = NG * NC

    def fwd_iter(n, gbase, st, filler=None):
        if n < NCH:
            g1, c1 = divmod(n, NC)
            if c1 == 0:
                st['qt'] = qt_s[gbase + g1]
                st['m'] = jnp.full((8, GW), -jnp.inf, f32)
            st['m'] = pass1_chunk(st['qt'], (sA, sB)[g1 % 2], c1, st['m'])
            if c1 == NC - 1:
                st['mdone'] = st['m']
        if filler is not None:
            filler()
        k = n - OFF
        if 0 <= k < NCH:
            g2, c2 = divmod(k, NC)
            if c2 == 0:
                st['mrow'] = jnp.max(st['mdone'], axis=0, keepdims=True)
                st['o'] = jnp.zeros((DH, GW), f32)
                st['l'] = jnp.zeros((8, GW), f32)
            st['o'], st['l'] = pass2_chunk(gbase + g2, (sA, sB)[g2 % 2], c2, st['mrow'], st['o'], st['l'])
            if c2 == NC - 1:
                linv = 1.0 / jnp.sum(st['l'], axis=0, keepdims=True)
                o_s[gbase + g2] = st['o'] * linv
                li_s[gbase + g2] = jnp.broadcast_to(linv, (8, GW))

    def fwd_dense(i):
        first = i == 0
        st = {}
        for n in range(2 * NC):
            fwd_iter(n, 0, st)

        def pack(st):
            return st['mdone'], jnp.broadcast_to(st['mrow'], (8, GW)), st['o'], st['l']

        def unpack(carry):
            st = dict(zip(('mdone', 'mrow', 'o', 'l'), carry))
            st['mrow'] = st['mrow'][0:1]
            return st

        def fbody(b, carry):
            st = unpack(carry)
            for n in range(2 * NC, 4 * NC):
                fwd_iter(n, 2 * b, st)
            return pack(st)
        st = unpack(lax.fori_loop(0, NG // 2 - 1, fbody, pack(st)))

        @pl.when(first)
        def _late_weights():
            for n in range(3, 8):
                in_copies[n].wait()
            woT[...] = wo_ref[...].T
            w2T[...] = w2_ref[...].T
            w1_s[...] = w1T[...].T
            w3_s[...] = w3T[...].T
            load_g(0)

        def dhh_piece(t):
            r0, r1 = t * 80, min(t * 80 + 80, F)
            dhh_s[r0:r1, :] = _dot(w2_ref[r0:r1, :], gt_s[...])
        for n in range(NCH, NCH + OFF):
            t = n - NCH
            fwd_iter(n, 0, st, filler=(lambda t=t: dhh_piece(t)) if t * 80 < F else None)

        _ungroup(ot_s, o_s, 1.0)
        z0 = jnp.minimum(i, 0)
        xt = x_ref[rows(i), :].astype(f32).T
        h = xt + _dot(woT[...], ot_s[...])
        h_s[z0] = h
        mean2 = _colmean(h)
        msq2 = _colmean(h * h)
        hnp_s[...] = hn_s[...]
        dx_q_part(jnp.maximum(i - 1, 0), first)
        accum(dw3_a, _dnt(du_s[...], hnp_s[...]), first)
        rstd2 = lax.rsqrt(jnp.maximum(msq2 - mean2 * mean2, 0.0) + EPS)
        hhat = (h_s[z0] - mean2) * rstd2
        hhat_s[...] = hhat
        hn_s[...] = hhat.astype(bf)

        for r0 in range(0, F, 128):
            r1 = min(r0 + 128, F)
            gate = _dot(w1T[r0:r1, :], hn_s[...])
            up = _dot(w3T[r0:r1, :], hn_s[...])
            dhh = dhh_s[r0:r1, :]
            sig = jax.nn.sigmoid(gate)
            silu = gate * sig
            hh_s[r0:r1, :] = (silu * up).astype(bf)
            du_s[r0:r1, :] = (dhh * silu).astype(bf)
            dg_s[r0:r1, :] = (dhh * up * (sig + silu * (1.0 - sig))).astype(bf)

        dhn = _dot(w1_s[...], dg_s[...]) + _dot(w3_s[...], du_s[...])
        dhn_s[z0] = dhn
        m1 = _colmean(dhn)
        m2 = _colmean(dhn * hhat_s[...])
        h2 = h_s[z0] + _dot(w2T[...], hh_s[...])
        h2_ref[i] = h2.astype(bf).T
        h2_copy(i).start()
        accum(dw2_a, _dnt(hh_s[...], gt_s[...]), first)
        for r0 in range(0, D, 128):
            rs = slice(r0, r0 + 128)
            dh = gt32_s[rs, :] + rstd2 * (dhn_s[z0, rs, :] - (hhat_s[rs, :] * m2 + m1))
            dh_s[i, rs, :] = dh
            dhb_s[rs, :] = dh.astype(bf)
        dO = _dot(wo_ref[...], dhb_s[...])
        accum(dwo_a, _dnt(ot_s[...], dhb_s[...]), first)
        accum(dw1_a, _dnt(dg_s[...], hn_s[...]), first)
        for g, dog in enumerate(_groups(dO)):
            dob = (dog * li_s[g, 0:1, :]).astype(bf)
            do_s[g] = dob
            dl_s[g] = jnp.broadcast_to(jnp.sum(dob.astype(f32) * o_s[g], axis=0, keepdims=True), (8, GW))

    def bwd(nxt):
        def A(g, dOg, delta, c, half):
            dp = _dot(vp_s[c, half * 64:half * 64 + 64, :], dOg)
            pa, pb = _unpack2(p_s[g, c * 64 + half * 32:c * 64 + half * 32 + 32, :])
            da, db = _split2(dp)
            ds_s[c % 4, half * 32:half * 32 + 32, :] = _pack2(pa * (da - delta), pb * (db - delta))

        def Bq(c, dq):
            return dq + _dot(kt_s[c], pltpu.bitcast(ds_s[c % 4], bf))

        def Bk(qt, c):
            dkt_s[c] += _dnt(qt, pltpu.bitcast(ds_s[c % 4], bf))

        def Bv(g, dOg, c):
            dvt_s[c] += _dnt(dOg, pltpu.bitcast(p_s[g, c * 64:(c + 1) * 64, :], bf))

        dq = prev = None
        for g in range(NG):
            qt, dOg, delta = qt_s[g], do_s[g], dl_s[g, 0:1, :]
            dq_new = jnp.zeros((DH, GW), f32)
            for it in range(NC):
                c = it - BLAG
                A(g, dOg, delta, it, 0)
                if c >= 0:
                    Bv(g, dOg, c)
                    dq_new = Bq(c, dq_new)
                elif g > 0:
                    Bv(g - 1, prev[1], NC + c)
                    dq = Bq(NC + c, dq)
                    if c == -1:
                        dq_s[g - 1] = dq
                A(g, dOg, delta, it, 1)
                if c >= 0:
                    Bk(qt, c)
                elif g > 0:
                    Bk(prev[0], NC + c)
            dq, prev = dq_new, (qt, dOg)
        for c in range(NC - BLAG, NC):
            Bv(NG - 1, prev[1], c)
            Bk(prev[0], c)
            dq = Bq(c, dq)
        dq_s[NG - 1] = dq
        if nxt is not None:
            q_proj(nxt)
            load_g(nxt)
        _ungroup(dqt_s, dq_s, DH ** -0.5)

    for cp in x_copies:
        cp.start()
    for cp in in_copies[:3]:
        cp.start()
    dkt_s[...] = jnp.zeros(dkt_s.shape, f32)
    dvt_s[...] = jnp.zeros(dvt_s.shape, f32)
    for n in range(XCH):
        x_copies[n].wait()
        if n == XCH - 1:
            for cp in in_copies[3:]:
                cp.start()
        for j in range(n * (NQ // XCH), (n + 1) * (NQ // XCH)):
            xt = x_ref[rows(j), :].astype(f32).T
            mean = _colmean(xt)
            rstd = lax.rsqrt(jnp.maximum(_colmean(xt * xt) - mean * mean, 0.0) + EPS)
            xh = (xt - mean) * rstd
            xn_s[j] = xh.astype(bf)
            xh_s[j] = xh
            rs_s[j] = jnp.broadcast_to(rstd, (8, BQ))
    in_copies[0].wait()
    in_copies[1].wait()
    wkvT = jnp.concatenate([wkT_ref[...], wvT_ref[...]], axis=0)
    wkv_s[...] = wkvT.astype(f32).T.astype(bf)
    r = lax.broadcasted_iota(jnp.int32, (128, 128), 0)
    c = lax.broadcasted_iota(jnp.int32, (128, 128), 1)
    rr = r % 16
    perm = jnp.where(c == (r - rr) + jnp.where(rr < 8, 2 * rr, 2 * (rr - 8) + 1), 1.0, 0.0).astype(bf)
    for j in range(NC):
        kv = _dot(wkvT, xn_s[j]).astype(bf)
        kt_s[j] = kv[0:DH]
        vt_s[j] = kv[DH:2 * DH]
    for j in range(NC):
        kp_s[j] = _dnt(perm, kt_s[j]).astype(bf)
        vp_s[j] = _dnt(perm, vt_s[j]).astype(bf)
    in_copies[2].wait()
    wqT[...] = wq_ref[...].T
    q_proj(0)

    dqt_s[...] = jnp.zeros(dqt_s.shape, bf)
    hn_s[...] = jnp.zeros(hn_s.shape, bf)
    du_s[...] = jnp.zeros(du_s.shape, bf)

    def block(i, carry):
        fwd_dense(i)

        @pl.when(i == NQ - 1)
        def _ffn_grads_out():
            dwo_ref[...] = dwo_a[...].astype(bf)
            w_copies[0].start()
            dw1T_ref[...] = dw1_a[...].astype(bf)
            w_copies[1].start()
            dw2_ref[...] = dw2_a[...].astype(bf)
            w_copies[2].start()
            dw3T_ref[...] = (dw3_a[...] + _dnt(du_s[...], hn_s[...])).astype(bf)
            w_copies[3].start()

        bwd(jnp.minimum(i + 1, NQ - 1))
        return carry
    lax.fori_loop(0, NQ, block, 0)

    dx_q_part(NQ - 1, False)
    dwq_ref[...] = dwq_a[...].astype(bf)
    w_copies[4].start()

    wkv = wkv_s[...]

    def ep_mm(j, acc):
        dkv = jnp.concatenate([(dkt_s[j] * (1.0 / LOG2E)).astype(bf), dvt_s[j].astype(bf)], axis=0)
        dxq_s[j] = dxq_s[j] + _dot(wkv, dkv)
        return acc + _dnt(dkv, xn_s[j])

    def ep_vpu(j):
        dy, xh, rstd = dxq_s[j], xh_s[j], rs_s[j, 0:1, :]
        m1 = _colmean(dy)
        m2 = _colmean(dy * xh)
        dx = dh_s[j] + rstd * (dy - (xh * m2 + m1))
        dx_ref[j] = dx.astype(bf).T
        dx_copy(j).start()

    acc = ep_mm(1, ep_mm(0, jnp.zeros((2 * DH, D), f32)))
    for j in range(NQ):
        if j + 2 < NQ:
            acc = ep_mm(j + 2, acc)
        ep_vpu(j)
    dwkT_ref[...] = acc[0:DH].astype(bf)
    dwvT_ref[...] = acc[DH:2 * DH].astype(bf)
    w_copies[5].start()
    w_copies[6].start()
    for cp in w_copies:
        cp.wait()

    def wait_blk(j, carry):
        h2_copy(j).wait()
        dx_copy(j).wait()
        return carry
    lax.fori_loop(0, NQ, wait_blk, 0)


@jax.jit
def pallas_sequential_preLN__grouped_kv_mqa__glu_gated_swiglu__prompt_kernel(
    A_x: jax.Array,
    A_wq: jax.Array,
    A_wk: jax.Array,
    A_wv: jax.Array,
    A_wo: jax.Array,
    B_x: jax.Array,
    B_w1: jax.Array,
    B_w3: jax.Array,
    B_w2: jax.Array,
    grad_out: jax.Array,
):
    del B_x
    ins = (A_x.reshape(S, D), A_wq, A_wk.T, A_wv.T, A_wo, B_w1.T, B_w3.T, B_w2, grad_out.reshape(S, D))
    out_shapes = [(S, D), (S, D), (D, D), (DH, D), (DH, D), (D, D), (F, D), (F, D), (F, D)]
    V = pltpu.VMEM
    SEM = pltpu.SemaphoreType.DMA
    scratch = (
        [V(a.shape, bf) for a in ins]
        + [V((NQ, BQ, D), bf), V((NQ, BQ, D), bf)] + [V(s, bf) for s in out_shapes[2:]]
        + [SEM((8,)), SEM((NQ,)), SEM((NQ,)), SEM((7,)), SEM((XCH,))]
        + [V((D, D), bf), V((D, D), bf), V((D, F), bf), V((D, F), bf), V((D, F), bf), V((D, 2 * DH), bf)]
        + [V((NQ, D, BQ), bf), V((NC, 128, DH), bf), V((NC, 128, DH), bf), V((NC, DH, 128), bf), V((NC, DH, 128), bf)]
        + [V((S, GW), f32), V((S, GW), f32), V((NG, S // 2, GW), u32), V((4, 64, GW), u32),
           V((NG, DH, GW), bf), V((NG, DH, GW), bf), V((NG, 8, GW), f32), V((NG, DH, GW), f32),
           V((NG, 8, GW), f32), V((NG, DH, GW), f32), V((NC, DH, 128), f32), V((NC, DH, 128), f32)]
        + [V((NQ, D, BQ), f32), V((NQ, D, BQ), f32), V((NQ, D, BQ), f32), V((NQ, 8, BQ), f32)]
        + [V((D, BQ), bf), V((F, BQ), bf), V((F, BQ), bf), V((F, BQ), bf), V((F, BQ), f32), V((D, BQ), bf),
           V((D, BQ), f32), V((D, BQ), bf), V((D, BQ), f32), V((D, BQ), bf), V((D, BQ), bf), V((D, BQ), bf),
           V((1, D, BQ), f32), V((1, D, BQ), f32)]
        + [V((D, D), f32), V((D, D), f32), V((F, D), f32), V((F, D), f32), V((F, D), f32)]
    )
    outs = pl.pallas_call(
        _kernel,
        in_specs=[pl.BlockSpec(memory_space=pl.ANY) for _ in ins],
        out_specs=[pl.BlockSpec(memory_space=pl.ANY) for _ in out_shapes],
        out_shape=[jax.ShapeDtypeStruct(s, bf) for s in out_shapes],
        scratch_shapes=scratch,
        compiler_params=pltpu.CompilerParams(vmem_limit_bytes=120 * 1024 * 1024),
    )(*ins)
    return (outs[0].reshape(1, S, D), outs[1].reshape(1, S, D), outs[2], outs[3].T, outs[4].T, outs[5],
            outs[6].T, outs[7].T, outs[8])
```
